```python
import os as _os
_os.environ.setdefault('JAX_PLATFORMS', 'cpu')
import jax
import jax.numpy as jnp

def _softmax(x, axis=-1):
    return jax.nn.softmax(x, axis=axis)

def _gelu(x):
    return jax.nn.gelu(x, approximate=True)

def _silu(x):
    return jax.nn.silu(x)

def _sigmoid(x):
    return jax.nn.sigmoid(x)

def _layernorm(x, axis=-1, eps=1e-05):
    m = jnp.mean(x, axis=axis, keepdims=True)
    v = jnp.var(x, axis=axis, keepdims=True)
    return (x - m) / jnp.sqrt(v + eps)

def _scatter_add(tgt, idx, src, axis=0):
    return tgt.at[idx].add(src)

def _segment_sum(src, seg, n):
    return jax.ops.segment_sum(src, seg, n)

class _Rng:

    def __init__(self, key):
        self._k = key

    def _next(self):
        self._k, sub = jax.random.split(self._k)
        return sub

    def normal(self, shape):
        return jax.random.normal(self._next(), shape, dtype=jnp.bfloat16)

    def randint(self, lo, hi, shape):
        return jax.random.randint(self._next(), shape, lo, hi, dtype=jnp.int32)

    def uniform(self, shape, lo=0.0, hi=1.0):
        return jax.random.uniform(self._next(), shape, jnp.bfloat16, lo, hi)

    def permutation(self, n):
        return jax.random.permutation(self._next(), n)
kernel_name = 'gated_mix__memory_aug_recurrent_mem_tr__glu_gated_geglu__prompt'

def setup_inputs():
    _rng = _Rng(jax.random.key(int.from_bytes(__import__("os").urandom(4), "little")))
    _w = lambda a: (lambda t: t.astype(jnp.bfloat16) if jnp.issubdtype(t.dtype, jnp.floating) else t)(jnp.asarray(a))

    def _A_setup():
        B, S, Dm = (1, 2048, 640)
        H, Dh = (32, 128)
        M, seg = (8, 32)
        seg = min(seg, S)
        S = S // seg * seg
        return {'x': _w((lambda *s: _rng.normal(s) * 0.05)(B, S, Dm)), 'mem0': _w((lambda *s: _rng.normal(s) * 0.4)(B, M, Dm)), 'Wq': _w((lambda *s: _rng.normal(s) * 3.2)(Dm, H, Dh) * Dm ** (-0.5)), 'Wk': _w((lambda *s: _rng.normal(s) * 3.2)(Dm, H, Dh) * Dm ** (-0.5)), 'Wv': _w((lambda *s: _rng.normal(s) * 0.4)(Dm, H, Dh) * Dm ** (-0.5)), 'Wo': _w((lambda *s: _rng.normal(s) * 0.4)(H, Dh, Dm) * (H * Dh) ** (-0.5)), 'seg_len': seg}
    _A_in = _A_setup()

    def _B_setup():
        B, S, Dm, Df = (1, 2048, 640, 1728)
        return {'x': _w((lambda *s: _rng.normal(s) * 0.05)(B, S, Dm)), 'w_gate': _w((lambda *s: _rng.normal(s) * 1.6)(Dm, Df) * Dm ** (-0.5)), 'w_up': _w((lambda *s: _rng.normal(s) * 1.6)(Dm, Df) * Dm ** (-0.5)), 'w_down': _w((lambda *s: _rng.normal(s) * 1.6)(Df, Dm) * Df ** (-0.5))}
    _B_in = _B_setup()
    return {'A_x': _A_in['x'], 'A_mem0': _A_in['mem0'], 'A_Wq': _A_in['Wq'], 'A_Wk': _A_in['Wk'], 'A_Wv': _A_in['Wv'], 'A_Wo': _A_in['Wo'], 'A_seg_len': _A_in['seg_len'], 'B_x': _B_in['x'], 'B_w_gate': _B_in['w_gate'], 'B_w_up': _B_in['w_up'], 'B_w_down': _B_in['w_down'], 'gate_w': _w((lambda *s: _rng.normal(s) * 0.05)(640) * 16.0)}

def reference(A_x, A_mem0, A_Wq, A_Wk, A_Wv, A_Wo, A_seg_len, B_x, B_w_gate, B_w_up, B_w_down, gate_w):

    def _A_ref(x, mem0, Wq, Wk, Wv, Wo, seg_len):
        B, S, Dm = x.shape
        H, Dh = (Wq.shape[1], Wq.shape[2])
        M = mem0.shape[1]
        scale = Dh ** (-0.5)
        n_seg = S // seg_len
        L = M + seg_len
        idx = jnp.arange(L)
        mask = (idx[:, None] < M) | (idx[:, None] >= idx[None, :])
        mem = mem0
        outs = []
        for s in range(n_seg):
            xs = x[:, s * seg_len:(s + 1) * seg_len, :].copy()
            h = jnp.concatenate([mem, xs], axis=1)
            q = jnp.einsum('btd,dhe->bhte', h, Wq)
            k = jnp.einsum('btd,dhe->bhte', h, Wk)
            v = jnp.einsum('btd,dhe->bhte', h, Wv)
            scores = jnp.einsum('bhqe,bhke->bhqk', q, k) * scale
            scores = jnp.where(mask[None, None], scores, -1000000000.0)
            p = _softmax(scores, axis=-1)
            o = jnp.einsum('bhqk,bhke->bhqe', p, v)
            o = jnp.einsum('bhte,hed->btd', o, Wo)
            mem = o[:, :M, :].copy()
            outs.append(o[:, M:, :])
        return jnp.concatenate(outs, axis=1)

    def _B_ref(x, w_gate, w_up, w_down):
        g = jnp.einsum('bsd,df->bsf', x, w_gate)
        u = jnp.einsum('bsd,df->bsf', x, w_up)
        h = _gelu(g) * u
        return jnp.einsum('bsf,fd->bsd', h, w_down)
    x = A_x
    g = _sigmoid((x * gate_w).sum(-1, keepdims=True))
    a = _A_ref(x, A_mem0, A_Wq, A_Wk, A_Wv, A_Wo, A_seg_len)
    b = _B_ref(x, B_w_gate, B_w_up, B_w_down)
    return g * a + (1 - g) * b
```

```python
import functools

import jax
import jax.numpy as jnp
import jax.experimental.pallas as pl
import jax.experimental.pallas.tpu as pltpu

F32 = jnp.float32
BF16 = jnp.bfloat16
U32 = jnp.uint32

LAGS_A = (1, 2)
LAGS_B = (1, 2)
WO_PER_TAIL = 2
WOC = 4
HB = 256
R0 = 448
RB = 240
NB = 6
NCUR = 4
ORDER = (6, 0, 1, 2, 3, 4, 5)
HS = 328


def _gelu_tanh(x):
    c = 0.7978845608028654
    return 0.5 * x * (1.0 + jnp.tanh(c * (x + 0.044715 * (x * x * x))))


def _dot(a, b):
    return jnp.dot(a, b, preferred_element_type=F32)


def _dot_t(a, b):
    return jax.lax.dot_general(a, b, (((1,), (1,)), ((), ())), preferred_element_type=F32)


def _pins(y, n):
    nr, nt = y.shape[0] // 8, y.shape[1] // 128
    out = []
    for i in range(n):
        k = (i * nr * nt) // n
        t, rr = k // nr, k % nr
        z = pltpu.bitcast(y[rr * 8:(rr + 1) * 8, t * 128:(t + 1) * 128], jnp.int32)
        z = jax.lax.shift_right_arithmetic(z, 31) + jax.lax.shift_right_logical(z, 31)
        out.append(pltpu.bitcast(z, U32))
    return out


def _kernel(x_hbm, mem0_hbm, wq_hbm, wk_hbm, wv_hbm, wo_hbm, wg_hbm, wu_hbm, wd_hbm, gw_hbm,
            out_hbm,
            x_v, mem0_v, st_v, wqkv_v, wo_v, wop_v, wgu_v, wd_v, gw_v,
            h_v, hc_v, b_v, q2_v, qc_v, kv_v, o_v, osave_v, out_v, sems,
            *, S, D, H, E, M, SEG, DF):
    n_pairs = S // (2 * SEG)
    scale = float(E) ** -0.5
    W = M + SEG + M
    R1 = R0 + NB * RB
    n_full = DF // HB
    rem = DF - n_full * HB
    assert rem == 192 and R1 < S and (S - R1) % 16 == 0
    n_hb = n_full + 1
    DH = D // 2
    NP = D // 2

    sem_ctr = [0]

    def dma(src, dst):
        c = pltpu.make_async_copy(src, dst, sems.at[sem_ctr[0]])
        sem_ctr[0] += 1
        c.start()
        return c

    RH = R0 // 2
    c_first = []
    for k in range(2):
        c_first.append([
            dma(x_hbm.at[k * RH:(k + 1) * RH], x_v.at[k * RH:(k + 1) * RH]),
            dma(wg_hbm.at[k * 128:(k + 1) * 128], wgu_v.at[k * 128:(k + 1) * 128]),
            dma(wu_hbm.at[k * 128:(k + 1) * 128], wgu_v.at[HB + k * 128:HB + (k + 1) * 128]),
        ])
    c_hb = [[]]
    for b in range(1, n_full):
        c_hb.append([
            dma(wg_hbm.at[b * HB:(b + 1) * HB], wgu_v.at[2 * b * HB:2 * b * HB + HB]),
            dma(wu_hbm.at[b * HB:(b + 1) * HB], wgu_v.at[2 * b * HB + HB:2 * (b + 1) * HB]),
        ])
    t0, u0 = n_full * HB, 2 * n_full * HB
    c_hb.append([
        dma(wg_hbm.at[t0:t0 + 128], wgu_v.at[u0:u0 + 128]),
        dma(wu_hbm.at[t0:t0 + 128], wgu_v.at[u0 + 128:u0 + 256]),
        dma(wg_hbm.at[t0 + 128:t0 + 192], wgu_v.at[u0 + 256:u0 + 320]),
        dma(wu_hbm.at[t0 + 128:t0 + 192], wgu_v.at[u0 + 320:u0 + 384]),
    ])
    c_gw = dma(gw_hbm, gw_v)
    c_mem = dma(mem0_hbm, mem0_v)
    st_sem0 = sem_ctr[0]
    for m, w_hbm in enumerate((wq_hbm, wk_hbm, wv_hbm)):
        for half in range(2):
            j = 2 * m + half
            dma(x_hbm.at[R0 + j * RB:R0 + (j + 1) * RB], x_v.at[R0 + j * RB:R0 + (j + 1) * RB])
            dma(w_hbm.at[half * DH * H:(half + 1) * DH * H], st_v.at[j])
    c_x1 = dma(x_hbm.at[R1:S], x_v.at[R1:S])
    c_wo = dma(wo_hbm, wo_v)
    c_wd = dma(wd_hbm, wd_v)
    out_sem = sem_ctr[0]

    def ffn_up(r0, n, b, ks=tuple(range(HB // 128))):
        xb = x_v[pl.ds(r0, n), :]
        if b < n_full:
            ys = []
            for k in ks:
                g0 = 2 * b * HB + k * 128
                yg = _dot_t(xb, wgu_v[g0:g0 + 128, :])
                yu = _dot_t(xb, wgu_v[g0 + HB:g0 + HB + 128, :])
                h_v[pl.ds(r0, n), b * HB + k * 128:b * HB + (k + 1) * 128] = (_gelu_tanh(yg) * yu).astype(BF16)
                ys += [yg, yu]
            y = jnp.concatenate(ys, axis=1)
        else:
            y = _dot_t(xb, wgu_v[u0:u0 + 2 * rem, :])
            h_v[pl.ds(r0, n), t0:t0 + 128] = (_gelu_tanh(y[:, 0:128]) * y[:, 128:256]).astype(BF16)
            h_v[pl.ds(r0, n), t0 + 128:t0 + 192] = (_gelu_tanh(y[:, 256:320]) * y[:, 320:384]).astype(BF16)
        return y

    def ffn_down(c):
        b_v[:, c * 128:(c + 1) * 128] = _dot(pltpu.bitcast(hc_v[...], BF16), wd_v[:, c * 128:(c + 1) * 128])

    def hc_copy(r, i, y=None):
        w = pltpu.bitcast(h_v[pl.ds(pl.multiple_of(r + 16 * i, 16), 16), :], U32)
        if y is not None:
            pins = _pins(y, -(-DF // 128))
            w = w | jnp.concatenate(pins, axis=1)[:, 0:DF]
        hc_v[8 * i:8 * (i + 1), :] = w

    RQ = R0 // 4
    for c in c_first[0]:
        c.wait()
    for k in range(2):
        ffn_up(k * RQ, RQ, 0, ks=(0,))
    for c in c_first[1]:
        c.wait()
    for k in range(2, 4):
        ffn_up(k * RQ, RQ, 0, ks=(0,))
    for k in range(4):
        ffn_up(k * RQ, RQ, 0, ks=(1,))
    for grp in ((1,), (2, 3), (6, 4, 5)):
        for b in grp:
            for c in c_hb[b]:
                c.wait()
        for b in grp:
            for k in range(4):
                ffn_up(k * (R0 // 4), R0 // 4, b)
    c_mem.wait()
    c_gw.wait()

    def ffn_relayout_body(j, carry):
        r0 = pl.multiple_of(R0 + j * RB, 16)
        xj = x_v.at[pl.ds(r0, RB)]
        pltpu.make_async_copy(xj, xj, sems.at[st_sem0 + 2 * j]).wait()
        pltpu.make_async_copy(st_v.at[j], st_v.at[j], sems.at[st_sem0 + 2 * j + 1]).wait()
        base0 = (j // 2) * (H * HS) + (j % 2) * (DH // 2)
        units = list(range(DH // 2))
        per = -(-len(units) // (n_hb - 1))

        def relayout(us, pins):
            for u, pin in zip(us, pins):
                blk = pltpu.bitcast(st_v[j, u * 2 * H:(u + 1) * 2 * H, :], U32)
                for half in range(2):
                    a = blk[half * 8:(half + 1) * 8] | pin
                    bb = blk[H // 2 + half * 8:H // 2 + (half + 1) * 8]
                    lo = (a & jnp.uint32(0xFFFF)) | (bb << 16)
                    hi = (a >> 16) | (bb & jnp.uint32(0xFFFF0000))
                    base = base0 + (half * 8 * HS + u)
                    wqkv_v[pl.ds(base, 8, stride=HS), :] = lo
                    wqkv_v[pl.ds(base + (H // 2) * HS, 8, stride=HS), :] = hi

        for b, blk_id in enumerate(ORDER):
            y = ffn_up(r0, RB, blk_id)
            us = units[b * per:(b + 1) * per]
            relayout(us, _pins(y, len(us)))
        return carry

    jax.lax.fori_loop(0, NB, ffn_relayout_body, 0)

    c_x1.wait()
    c_wo.wait()
    c_wd.wait()
    for i in range(2 * SEG // 16):
        hc_copy(0, i)
    n_wo = H * E // 16
    per_wo = -(-n_wo // (n_hb - 1))
    for b, blk_id in enumerate(ORDER):
        y = ffn_up(R1, S - R1, blk_id)
        us = list(range(b * per_wo, min((b + 1) * per_wo, n_wo)))
        for i, pin in zip(us, _pins(y, len(us))):
            w = pltpu.bitcast(wo_v[i * 16:(i + 1) * 16, :], U32)
            wop_v[i * 8:(i + 1) * 8, :] = w | jnp.concatenate([pin] * (D // 128), axis=1)
    for c in range(NCUR, D // 128):
        ffn_down(c)

    def w_head(m, h):
        p = (m * H + (h % 2) * (H // 2) + h // 2) * HS
        return pltpu.bitcast(wqkv_v[p:p + NP, :], BF16)

    L = M + SEG
    r = jax.lax.broadcasted_iota(jnp.int32, (2 * L, 2 * W), 0)
    cc = jax.lax.broadcasted_iota(jnp.int32, (2 * L, 2 * W), 1)
    same = (r >= L) == (cc >= W)
    r = jnp.where(r >= L, r - L, r)
    cc = jnp.where(cc >= W, cc - W, cc)
    real_a = same & (cc < L)
    mask_a = real_a & ((r < M) | (r >= cc))

    def logical(w):
        return jnp.where(w < 2 * M, w, jnp.where(w < 3 * M, w - 2 * M, w - M))
    lr, lc = logical(r + M), logical(cc)
    real_b = same & (cc >= M)
    mask_b = real_b & ((lr < M) | (lr >= lc))
    fill_a = jnp.where(real_a, -1e9, -jnp.inf).astype(F32)
    fill_b = jnp.where(real_b, -1e9, -jnp.inf).astype(F32)
    HP = H // 2

    def step(lhs, row0, win0, mask, fill, first, fillers):
        nrows = lhs.shape[0]
        nwo = SEG if first else W
        L1, L2 = LAGS_A if first else LAGS_B
        pend = {}

        def st_qkv(i):
            y0 = _dot(lhs, w_head(0, 2 * i))
            y1 = _dot(lhs, w_head(0, 2 * i + 1))
            if first:
                q2 = jnp.concatenate([y0[0:L], y1[0:L]], axis=0)
                qc_v[i] = jnp.concatenate([y0[L:W], y1[L:W]], axis=0)
            else:
                qc = qc_v[i]
                q2 = jnp.concatenate([qc[0:M], y0, qc[M:2 * M], y1], axis=0)
            q2_v[i] = q2.astype(BF16)
            for m in range(2):
                for j in range(2):
                    y = _dot(lhs, w_head(m + 1, 2 * i + j))
                    kv_v[m * H + 2 * i + j, row0:row0 + nrows, :] = y.astype(BF16)

        def kv2(m, i):
            return jnp.concatenate([kv_v[m * H + 2 * i + j, win0:win0 + W, :] for j in range(2)], axis=0)

        def st_scores(i):
            s = _dot_t(q2_v[i], kv2(0, i)) * scale
            s = jnp.where(mask, s, fill)
            mx = jnp.max(s, axis=-1, keepdims=True)
            p = jnp.exp(s - mx)
            l = jnp.sum(p, axis=-1, keepdims=True)
            rl = pl.reciprocal(l, approx=True)
            rl = rl * (2.0 - l * rl)
            pend[i] = (p * rl).astype(BF16)

        def st_pv(i):
            o2 = _dot(pend.pop(i), kv2(1, i))
            for j in range(2):
                h = 2 * i + j
                o = o2[j * L:(j + 1) * L]
                if first:
                    o_v[0:SEG, h * E:(h + 1) * E] = o[0:SEG].astype(BF16)
                    osave_v[:, h * E:(h + 1) * E] = o[SEG:L]
                else:
                    o = jnp.concatenate([osave_v[:, h * E:(h + 1) * E], o], axis=0)
                    o_v[:, h * E:(h + 1) * E] = o.astype(BF16)

        acc = [None]

        def st_wo(c):
            lo, hi = c * WOC * E, (c + 1) * WOC * E
            y = _dot(o_v[0:nwo, lo:hi], pltpu.bitcast(wop_v[lo // 2:hi // 2, :], BF16))
            acc[0] = y if acc[0] is None else acc[0] + y
            if c in fillers.get("wo", {}):
                fillers["wo"][c](y)

        nxt_wo = 0
        for i in range(HP + L1 + L2):
            for f in fillers.get(i, ()):
                f()
            if i < HP:
                st_qkv(i)
            else:
                for _ in range(WO_PER_TAIL):
                    if (nxt_wo + 1) * WOC <= 2 * (i - L1 - L2):
                        st_wo(nxt_wo)
                        nxt_wo += 1
            if 0 <= i - L1 < HP:
                st_scores(i - L1)
            if 0 <= i - L1 - L2 < HP:
                st_pv(i - L1 - L2)
        while nxt_wo < H // WOC:
            st_wo(nxt_wo)
            nxt_wo += 1
        for f in fillers.get("end", ()):
            f()
        return acc[0]

    def pair_body(t, mem):
        r0 = pl.multiple_of(t * (2 * SEG), 2 * SEG)
        rn = pl.multiple_of(jnp.minimum(r0 + 2 * SEG, S - 2 * SEG), 2 * SEG)
        dn = [functools.partial(ffn_down, c) for c in range(D // 128)]
        work_a = {HP: dn[0:1], "end": dn[1:NCUR]}
        work_b = {"wo": {2 + i: functools.partial(hc_copy, rn, i) for i in range(2 * SEG // 16)}}

        xx = x_v[pl.ds(r0, 2 * SEG), :].astype(F32)
        lhs_a = jnp.concatenate([mem, xx[0:SEG + M]], axis=0).astype(BF16)
        out_a = step(lhs_a, 0, 0, mask_a, fill_a, True, work_a)
        mem_b = out_a[0:M]
        lhs_b = jnp.concatenate([mem_b, xx[SEG + M:2 * SEG]], axis=0).astype(BF16)
        out_b = step(lhs_b, W, SEG, mask_b, fill_b, False, work_b)
        mem_n = out_b[2 * M:3 * M]
        a = jnp.concatenate([out_a[M:SEG], out_b[0:2 * M], out_b[3 * M:W]], axis=0)
        gw = gw_v[...].astype(F32).reshape(1, D)
        g = jax.nn.sigmoid(jnp.sum(xx * gw, axis=-1, keepdims=True))
        out_v[pl.ds(r0, 2 * SEG), :] = (g * a + (1.0 - g) * b_v[...]).astype(out_v.dtype)
        pltpu.make_async_copy(out_v.at[pl.ds(r0, 2 * SEG)], out_hbm.at[pl.ds(r0, 2 * SEG)],
                              sems.at[out_sem]).start()
        for f in dn[NCUR:]:
            f()
        return mem_n

    jax.lax.fori_loop(0, n_pairs, pair_body, mem0_v[...].astype(F32), unroll=2)

    pltpu.make_async_copy(out_v, out_hbm, sems.at[out_sem]).wait()


@functools.partial(jax.jit, static_argnames=("SEG",))
def _run(A_x, A_mem0, A_Wq, A_Wk, A_Wv, A_Wo, B_w_gate, B_w_up, B_w_down, gate_w, *, SEG):
    B, S, D = A_x.shape
    H, E = A_Wq.shape[1], A_Wq.shape[2]
    M = A_mem0.shape[1]
    DF = B_w_gate.shape[1]
    assert B == 1 and M == 8 and SEG == 32 and S % (2 * SEG) == 0 and E == 128 and H == 32

    x = A_x.reshape(S, D)
    mem0 = A_mem0.reshape(M, D)
    wq = A_Wq.reshape(D * H, E)
    wk = A_Wk.reshape(D * H, E)
    wv = A_Wv.reshape(D * H, E)
    wo = A_Wo.reshape(H * E, D)
    wgt = B_w_gate.T
    wut = B_w_up.T

    kern = functools.partial(_kernel, S=S, D=D, H=H, E=E, M=M, SEG=SEG, DF=DF)
    hbm_spec = pl.BlockSpec(memory_space=pltpu.HBM)
    out = pl.pallas_call(
        kern,
        out_shape=jax.ShapeDtypeStruct((S, D), A_x.dtype),
        in_specs=[hbm_spec] * 10,
        out_specs=hbm_spec,
        scratch_shapes=[
            pltpu.VMEM((S, D), BF16),
            pltpu.VMEM((M, D), BF16),
            pltpu.VMEM((6, D // 2 * H, E), BF16),
            pltpu.VMEM((3 * H * HS, E), U32),
            pltpu.VMEM((H * E, D), BF16),
            pltpu.VMEM((H * E // 2, D), U32),
            pltpu.VMEM((2 * DF, D), BF16),
            pltpu.VMEM((DF, D), BF16),
            pltpu.VMEM((D,), BF16),
            pltpu.VMEM((S, DF), BF16),
            pltpu.VMEM((SEG, DF), U32),
            pltpu.VMEM((2 * SEG, D), F32),
            pltpu.VMEM((H // 2, 2 * (M + SEG), E), BF16),
            pltpu.VMEM((H // 2, 2 * M, E), F32),
            pltpu.VMEM((2 * H, 2 * (M + SEG), E), BF16),
            pltpu.VMEM((M + SEG + M, H * E), BF16),
            pltpu.VMEM((M, H * E), F32),
            pltpu.VMEM((S, D), BF16),
            pltpu.SemaphoreType.DMA((48,)),
        ],
        compiler_params=pltpu.CompilerParams(vmem_limit_bytes=100 * 1024 * 1024),
    )(x, mem0, wq, wk, wv, wo, wgt, wut, B_w_down, gate_w)
    return out.reshape(B, S, D)


def pallas_gated_mix__memory_aug_recurrent_mem_tr__glu_gated_geglu__prompt_kernel(
    A_x: jax.Array,
    A_mem0: jax.Array,
    A_Wq: jax.Array,
    A_Wk: jax.Array,
    A_Wv: jax.Array,
    A_Wo: jax.Array,
    A_seg_len,
    B_x: jax.Array,
    B_w_gate: jax.Array,
    B_w_up: jax.Array,
    B_w_down: jax.Array,
    gate_w: jax.Array,
):
    seg = A_seg_len if isinstance(A_seg_len, int) else 32
    return _run(A_x, A_mem0, A_Wq, A_Wk, A_Wv, A_Wo, B_w_gate, B_w_up, B_w_down, gate_w, SEG=seg)
```
